```python
import os as _os
_os.environ.setdefault("JAX_PLATFORMS", "cpu")
import jax
import jax.numpy as jnp

def _softmax(x, axis=-1):
    return jax.nn.softmax(x, axis=axis)
def _gelu(x):
    return jax.nn.gelu(x, approximate=True)
def _silu(x):
    return jax.nn.silu(x)
def _sigmoid(x):
    return jax.nn.sigmoid(x)
def _layernorm(x, axis=-1, eps=1e-5):
    m = jnp.mean(x, axis=axis, keepdims=True)
    v = jnp.var(x, axis=axis, keepdims=True)
    return (x - m) / jnp.sqrt(v + eps)
def _scatter_add(tgt, idx, src, axis=0):
    return tgt.at[idx].add(src)
def _segment_sum(src, seg, n):
    return jax.ops.segment_sum(src, seg, n)
class _Rng:
    def __init__(self, key):
        self._k = key
    def _next(self):
        self._k, sub = jax.random.split(self._k)
        return sub
    def normal(self, shape):
        return jax.random.normal(self._next(), shape, dtype=jnp.bfloat16)
    def randint(self, lo, hi, shape):
        return jax.random.randint(self._next(), shape, lo, hi, dtype=jnp.int32)
    def uniform(self, shape, lo=0.0, hi=1.0):
        return jax.random.uniform(self._next(), shape, jnp.bfloat16, lo, hi)
    def permutation(self, n):
        return jax.random.permutation(self._next(), n)


kernel_name = 'interleave_layers__mha_block__dense_activation_mish__prompt'

def setup_inputs():
    _rng = _Rng(jax.random.key(int.from_bytes(__import__("os").urandom(4), "little")))
    _w = (lambda a: (lambda t: t.astype(jnp.bfloat16) if jnp.issubdtype(t.dtype, jnp.floating) else t)(jnp.asarray(a)))
    def _A_setup():
        B, S, D, H = 1, 2048, 512, 32
        return {
            "x": _w((lambda *s: _rng.normal(s) * 0.05)(B, S, D)),
            "wqkv": _w((lambda *s: _rng.normal(s) * 0.05)(D, 3 * D)),
            "wo": _w((lambda *s: _rng.normal(s) * 0.05)(D, D)),
        }
    _A_in = _A_setup()

    def _B_setup():
        B, S, D, F = 1, 2048, 512, 1792
        return {
            "x": _w((lambda *s: _rng.normal(s) * 0.05)(B, S, D)),
            "w1": _w((lambda *s: _rng.normal(s) * 0.4)(D, F) * (D ** -0.5)),
            "b1": _w((lambda *s: _rng.normal(s) * 0.4)(F)),
            "w2": _w((lambda *s: _rng.normal(s) * 0.4)(F, D) * (F ** -0.5)),
        }
    _B_in = _B_setup()

    return {
        "A_x": _A_in["x"],
        "A_wqkv": _A_in["wqkv"],
        "A_wo": _A_in["wo"],
        "B_x": _B_in["x"],
        "B_w1": _B_in["w1"],
        "B_b1": _B_in["b1"],
        "B_w2": _B_in["w2"],
    }

def reference(A_x, A_wqkv, A_wo, B_x, B_w1, B_b1, B_w2):
    def _A_ref(x, wqkv, wo):
        B, S, D = x.shape
        H = 32
        Dh = D // H
        qkv = (lambda x, *d: x.transpose(*d))((x @ wqkv).reshape(B, S, 3, H, Dh), 2, 0, 3, 1, 4)
        q, k, v = qkv[0], qkv[1], qkv[2]
        scores = jnp.einsum("bhqd,bhkd->bhqk", q, k) * (Dh ** -0.5)
        p = _softmax(scores, axis=-1)
        o = jnp.einsum("bhqk,bhkd->bhqd", p, v)
        return (lambda x, *d: x.transpose(*d))(o, 0, 2, 1, 3).reshape(B, S, D) @ wo

    def _B_ref(x, w1, b1, w2):
        h = jnp.einsum("bsd,df->bsf", x, w1) + b1
        sp = jnp.log1p(jnp.exp(-jnp.abs(h))) + jnp.where(h > 0, h, jnp.zeros_like(h))
        act = h * jnp.tanh(sp)
        return jnp.einsum("bsf,fd->bsd", act, w2)

    x = A_x
    x = x + _A_ref(_layernorm(x, axis=-1), A_wqkv, A_wo)
    x = x + _B_ref(_layernorm(x, axis=-1), B_w1, B_b1, B_w2)
    x = x + _A_ref(_layernorm(x, axis=-1), A_wqkv, A_wo)
    x = x + _B_ref(_layernorm(x, axis=-1), B_w1, B_b1, B_w2)
    return x
```

```python
import functools

import jax
import jax.numpy as jnp
import jax.experimental.pallas as pl
import jax.experimental.pallas.tpu as pltpu

S = 2048
D = 512
H = 32
DH = 16
F = 1792
EPS = 1e-5
LOG2E = 1.4426950408889634

TT = 512
TQ = 256
KC = 256
NB = 4
NQ = S // TQ
NC = S // KC
NIT = H * NQ

f32 = jnp.float32
bf16 = jnp.bfloat16


def _ln_t(x):
    m = jnp.mean(x, axis=0, keepdims=True)
    xc = x - m
    v = jnp.mean(xc * xc, axis=0, keepdims=True)
    return xc * jax.lax.rsqrt(v + EPS)


def _mish(h):
    sp = jnp.log1p(jnp.exp(-jnp.abs(h))) + jnp.maximum(h, 0.0)
    return h * jnp.tanh(sp)


def _kernel(x_ref, wqkv_ref, wo_ref, w1_ref, b1_ref, w2_ref, out_ref,
            xt_ref, wqkvt_ref, wot_ref, w1t_ref, w2t_ref, b1t_ref,
            qt_ref, k_ref, vt_ref, ot_ref, *s_refs):
    wqkvt_ref[...] = wqkv_ref[...].astype(f32).T.astype(bf16)
    wot_ref[...] = wo_ref[...].astype(f32).T.astype(bf16)
    w1t_ref[...] = w1_ref[...].astype(f32).T.astype(bf16)
    w2t_ref[...] = w2_ref[...].astype(f32).T.astype(bf16)
    b1t_ref[...] = jnp.broadcast_to(b1_ref[...].astype(f32), (128, F)).T
    for t in range(S // TT):
        xt_ref[:, t * TT:(t + 1) * TT] = x_ref[t * TT:(t + 1) * TT, :].astype(f32).T

    def qkv_tile(t, carry):
        cols = pl.ds(pl.multiple_of(t * TT, TT), TT)
        xn = _ln_t(xt_ref[:, cols]).astype(bf16)
        qkv = jnp.dot(wqkvt_ref[...], xn, preferred_element_type=f32)
        qt_ref[:, cols] = (qkv[0:D] * (DH ** -0.5 * LOG2E)).astype(bf16)
        k_ref[cols, :] = qkv[D:2 * D].T.astype(bf16)
        vt_ref[:, cols] = qkv[2 * D:3 * D].astype(bf16)
        return carry

    def post_tile(t, carry):
        cols = pl.ds(pl.multiple_of(t * TT, TT), TT)
        x = xt_ref[:, cols] + jnp.dot(wot_ref[...], ot_ref[:, cols],
                                      preferred_element_type=f32)
        xn = _ln_t(x).astype(bf16)
        b = b1t_ref[...]
        h = jnp.dot(w1t_ref[...], xn, preferred_element_type=f32)
        h = h + jnp.concatenate([b] * (TT // 128), axis=1)
        act = _mish(h).astype(bf16)
        xt_ref[:, cols] = x + jnp.dot(w2t_ref[...], act, preferred_element_type=f32)
        return carry

    def masked_q(h, qt):
        g = h // 8
        j = h % 8
        qg = qt_ref[pl.ds(pl.multiple_of(g * 128, 128), 128),
                    pl.ds(pl.multiple_of(qt * TQ, TQ), TQ)]
        rows = jax.lax.broadcasted_iota(jnp.int32, (128, TQ), 0)
        msk = (rows >= j * DH) & (rows < j * DH + DH)
        return jnp.where(msk, qg, jnp.zeros_like(qg))

    def fused(it, m_cur, s_cur, s_nxt, dist, do2=True):
        h = it // NQ
        qt = it % NQ
        itn = jnp.minimum(it + dist, NIT - 1)
        hn = itn // NQ
        qtn = itn % NQ
        gn = hn // 8
        qm = masked_q(hn, qtn)
        m = jnp.full((1, TQ), -jnp.inf, f32)
        o = jnp.zeros((DH, TQ), f32)
        l = jnp.zeros((1, TQ), f32)
        for c in range(NC):
            kg = k_ref[pl.ds(c * KC, KC), pl.ds(pl.multiple_of(gn * 128, 128), 128)]
            s = jnp.dot(kg, qm, preferred_element_type=f32)
            s_nxt[pl.ds(c * KC, KC), :] = s
            m = jnp.maximum(m, jnp.max(s, axis=0, keepdims=True))
            if do2:
                pf = jnp.exp2(s_cur[pl.ds(c * KC, KC), :] - m_cur)
                l = l + jnp.sum(pf, axis=0, keepdims=True)
                o = o + jnp.dot(vt_ref[pl.ds(pl.multiple_of(h * DH, DH), DH), pl.ds(c * KC, KC)],
                                pf.astype(bf16), preferred_element_type=f32)
        if do2:
            ot_ref[pl.ds(pl.multiple_of(h * DH, DH), DH),
                   pl.ds(pl.multiple_of(qt * TQ, TQ), TQ)] = (o / l).astype(bf16)
        return m

    def attention():
        dist = NB - 1
        ms = []
        for b in range(dist):
            ms.append(fused(b - dist, None, None, s_refs[b], dist, do2=False))

        def body(ib, ms):
            ms = list(ms)
            for u in range(NB):
                it = ib * NB + u
                mnew = fused(it, ms[0], s_refs[u % NB], s_refs[(u + dist) % NB], dist)
                ms = ms[1:] + [mnew]
            return tuple(ms)

        jax.lax.fori_loop(0, NIT // NB, body, tuple(ms))

    def layer(l, carry):
        jax.lax.fori_loop(0, S // TT, qkv_tile, 0)
        attention()
        jax.lax.fori_loop(0, S // TT, post_tile, 0)
        return carry

    jax.lax.fori_loop(0, 2, layer, 0)

    for t in range(S // TT):
        out_ref[t * TT:(t + 1) * TT, :] = xt_ref[:, t * TT:(t + 1) * TT].T.astype(bf16)


@jax.jit
def pallas_interleave_layers__mha_block__dense_activation_mish__prompt_kernel(
    A_x: jax.Array,
    A_wqkv: jax.Array,
    A_wo: jax.Array,
    B_x: jax.Array,
    B_w1: jax.Array,
    B_b1: jax.Array,
    B_w2: jax.Array,
):
    x = A_x.reshape(S, D)
    b1 = B_b1.reshape(1, F)
    out = pl.pallas_call(
        _kernel,
        out_shape=jax.ShapeDtypeStruct((S, D), bf16),
        scratch_shapes=[
            pltpu.VMEM((D, S), f32),
            pltpu.VMEM((3 * D, D), bf16),
            pltpu.VMEM((D, D), bf16),
            pltpu.VMEM((F, D), bf16),
            pltpu.VMEM((D, F), bf16),
            pltpu.VMEM((F, 128), f32),
            pltpu.VMEM((D, S), bf16),
            pltpu.VMEM((S, D), bf16),
            pltpu.VMEM((D, S), bf16),
            pltpu.VMEM((D, S), bf16),
        ] + [pltpu.VMEM((S, TQ), f32) for _ in range(NB)],
        compiler_params=pltpu.CompilerParams(vmem_limit_bytes=100 * 1024 * 1024),
    )(x, A_wqkv, A_wo, B_w1, b1, B_w2)
    return out.reshape(1, S, D)
```

```python
import functools

import jax
import jax.numpy as jnp
import jax.experimental.pallas as pl
import jax.experimental.pallas.tpu as pltpu

S = 2048
D = 512
H = 32
DH = 16
F = 1792
EPS = 1e-5
LOG2E = 1.4426950408889634

TT = 512
TQ = 256
KC = 256
NB = 8
PEEL = True

f32 = jnp.float32
bf16 = jnp.bfloat16


def _ln_t(x):
    m = jnp.mean(x, axis=0, keepdims=True)
    xc = x - m
    v = jnp.mean(xc * xc, axis=0, keepdims=True)
    return xc * jax.lax.rsqrt(v + EPS)


def _mish(h):
    sp = jnp.log1p(jnp.exp(-jnp.abs(h))) + jnp.maximum(h, 0.0)
    return h * jnp.tanh(sp)


def _kernel(x_hbm, wqkv_hbm, wo_hbm, w1_hbm, b1_hbm, w2_hbm, out_hbm,
            x_ref, wqkv_ref, wo_ref, w1_ref, b1_ref, w2_ref, in_sems, out_sems,
            xt_ref, wqkvt_ref, wot_ref, w1t_ref, w2t_ref, b1t_ref,
            qt_ref, k_ref, vt_ref, ot_ref, *s_refs):
    NQ = S // TQ
    NC = S // KC
    NIT = H * NQ
    NT = S // TT

    in_copies = [
        pltpu.make_async_copy(src, dst, in_sems.at[i])
        for i, (src, dst) in enumerate([
            (x_hbm, x_ref), (wqkv_hbm, wqkv_ref), (wo_hbm, wo_ref),
            (w1_hbm, w1_ref), (b1_hbm, b1_ref), (w2_hbm, w2_ref)])
    ]
    for cp in in_copies:
        cp.start()

    def out_copy(t):
        rows = pl.ds(pl.multiple_of(t * TT, TT), TT)
        return pltpu.make_async_copy(x_ref.at[rows, :], out_hbm.at[rows, :], out_sems.at[t])

    def qkv_tile(t, carry):
        cols = pl.ds(pl.multiple_of(t * TT, TT), TT)
        xn = _ln_t(xt_ref[:, cols]).astype(bf16)
        qkv = jnp.dot(wqkvt_ref[...], xn, preferred_element_type=f32)
        qt_ref[:, cols] = (qkv[0:D] * (DH ** -0.5 * LOG2E)).astype(bf16)
        k_ref[cols, :] = qkv[D:2 * D].T.astype(bf16)
        vt_ref[:, cols] = qkv[2 * D:3 * D].astype(bf16)
        return carry

    def post_tile(t, layer):
        cols = pl.ds(pl.multiple_of(t * TT, TT), TT)
        x = xt_ref[:, cols] + jnp.dot(wot_ref[...], ot_ref[:, cols],
                                      preferred_element_type=f32)
        xn = _ln_t(x).astype(bf16)
        b = b1t_ref[...]
        h = jnp.dot(w1t_ref[...], xn, preferred_element_type=f32)
        h = h + jnp.concatenate([b] * (TT // 128), axis=1)
        act = _mish(h).astype(bf16)
        xt_ref[:, cols] = x + jnp.dot(w2t_ref[...], act, preferred_element_type=f32)

        @pl.when(layer == 1)
        def _():
            x_ref[cols, :] = xt_ref[:, cols].T.astype(bf16)
            out_copy(t).start()
        return layer

    def fused(ib, u, m_cur, s_buf, do1=True, do2=True):
        GB = H // NB
        h = (ib % GB) * NB + u
        qt = ib // GB
        hn = ((ib + 1) % GB) * NB + u
        qtn = (ib + 1) // GB
        gn = ((ib + 1) % GB) * NB // 8
        jn = u % 8
        if do1:
            qm = qt_ref[pl.ds(pl.multiple_of(hn * DH, DH), DH),
                        pl.ds(pl.multiple_of(qtn * TQ, TQ), TQ)]
        m = jnp.full((1, TQ), -jnp.inf, f32)
        o = jnp.zeros((DH, TQ), f32)
        l = jnp.zeros((1, TQ), f32)
        for c in range(NC):
            if do2:
                pf = jnp.exp2(s_buf[pl.ds(c * KC, KC), :] - m_cur)
                l = l + jnp.sum(pf, axis=0, keepdims=True)
                o = o + jnp.dot(vt_ref[pl.ds(pl.multiple_of(h * DH, DH), DH), pl.ds(c * KC, KC)],
                                pf.astype(bf16), preferred_element_type=f32)
            if do1:
                kg = k_ref[pl.ds(c * KC, KC), pl.ds(pl.multiple_of(gn * 128, 128), 128)]
                kg = kg[:, jn * DH:(jn + 1) * DH]
                s = jnp.dot(kg, qm, preferred_element_type=f32)
                s_buf[pl.ds(c * KC, KC), :] = s
                m = jnp.maximum(m, jnp.max(s, axis=0, keepdims=True))
        if do2:
            ot_ref[pl.ds(pl.multiple_of(h * DH, DH), DH),
                   pl.ds(pl.multiple_of(qt * TQ, TQ), TQ)] = (o / l).astype(bf16)
        return m

    def attention():
        ms = []
        for b in range(NB):
            ms.append(fused(-1, b, None, s_refs[b], do2=False))
        wot_ref[...] = wo_ref[...].astype(f32).T.astype(bf16)
        w1t_ref[...] = w1_ref[...].astype(f32).T.astype(bf16)
        w2t_ref[...] = w2_ref[...].astype(f32).T.astype(bf16)
        b1t_ref[...] = jnp.broadcast_to(b1_ref[...].astype(f32), (128, F)).T

        def body(ib, ms):
            return tuple(fused(ib, u, ms[u], s_refs[u]) for u in range(NB))

        if PEEL:
            ms = jax.lax.fori_loop(0, NIT // NB - 1, body, tuple(ms))
            for u in range(NB):
                fused(NIT // NB - 1, u, ms[u], s_refs[u], do1=False)
        else:
            jax.lax.fori_loop(0, NIT // NB, body, tuple(ms))

    in_copies[0].wait()
    for t in range(NT):
        xt_ref[:, t * TT:(t + 1) * TT] = x_ref[t * TT:(t + 1) * TT, :].astype(f32).T
    in_copies[1].wait()
    wqkvt_ref[...] = wqkv_ref[...].astype(f32).T.astype(bf16)

    def layer_fn(layer, carry):
        jax.lax.fori_loop(0, NT, qkv_tile, 0)

        @pl.when(layer == 0)
        def _():
            in_copies[2].wait()
            in_copies[3].wait()
            in_copies[4].wait()
            in_copies[5].wait()

        attention()
        jax.lax.fori_loop(0, NT, post_tile, layer)
        return carry

    jax.lax.fori_loop(0, 2, layer_fn, 0)
    for t in range(NT):
        out_copy(t).wait()


@jax.jit
def pallas_interleave_layers__mha_block__dense_activation_mish__prompt_kernel(
    A_x: jax.Array,
    A_wqkv: jax.Array,
    A_wo: jax.Array,
    B_x: jax.Array,
    B_w1: jax.Array,
    B_b1: jax.Array,
    B_w2: jax.Array,
):
    x = A_x.reshape(S, D)
    b1 = B_b1.reshape(1, F)
    out = pl.pallas_call(
        _kernel,
        out_shape=jax.ShapeDtypeStruct((S, D), bf16),
        in_specs=[pl.BlockSpec(memory_space=pl.ANY)] * 6,
        out_specs=pl.BlockSpec(memory_space=pl.ANY),
        scratch_shapes=[
            pltpu.VMEM((S, D), bf16),
            pltpu.VMEM((D, 3 * D), bf16),
            pltpu.VMEM((D, D), bf16),
            pltpu.VMEM((D, F), bf16),
            pltpu.VMEM((1, F), bf16),
            pltpu.VMEM((F, D), bf16),
            pltpu.SemaphoreType.DMA((6,)),
            pltpu.SemaphoreType.DMA((S // TT,)),
            pltpu.VMEM((D, S), f32),
            pltpu.VMEM((3 * D, D), bf16),
            pltpu.VMEM((D, D), bf16),
            pltpu.VMEM((F, D), bf16),
            pltpu.VMEM((D, F), bf16),
            pltpu.VMEM((F, 128), f32),
            pltpu.VMEM((D, S), bf16),
            pltpu.VMEM((S, D), bf16),
            pltpu.VMEM((D, S), bf16),
            pltpu.VMEM((D, S), bf16),
        ] + [pltpu.VMEM((S, TQ), f32) for _ in range(NB)],
        compiler_params=pltpu.CompilerParams(vmem_limit_bytes=100 * 1024 * 1024),
    )(x, A_wqkv, A_wo, B_w1, b1, B_w2)
    return out.reshape(1, S, D)
```

```python
import jax
import jax.numpy as jnp
import jax.experimental.pallas as pl
import jax.experimental.pallas.tpu as pltpu

S = 2048
D = 512
H = 32
DH = 16
F = 1792
EPS = 1e-5
LOG2E = 1.4426950408889634

TT = 1024
TQ = 256
KC = 256
NB = 8

f32 = jnp.float32
bf16 = jnp.bfloat16


def _ln_t(x):
    m = jnp.mean(x, axis=0, keepdims=True)
    xc = x - m
    v = jnp.mean(xc * xc, axis=0, keepdims=True)
    return xc * jax.lax.rsqrt(v + EPS)


def _mish(h):
    sp = jnp.log1p(jnp.exp(-jnp.abs(h))) + jnp.maximum(h, 0.0)
    return h * jnp.tanh(sp)


def _kernel(x_hbm, wqkv_hbm, wo_hbm, w1_hbm, b1_hbm, w2_hbm, out_hbm,
            x_ref, wqkv_ref, wo_ref, w1_ref, b1_ref, w2_ref, in_sems, out_sems,
            xt_ref, wqkvt_ref, wot_ref, w1t_ref, w2t_ref, b1t_ref,
            qt_ref, k_ref, vt_ref, ot_ref, *s_refs):
    NQ = S // TQ
    NC = S // KC
    NT = S // TT
    GB = H // NB
    NBODY = NQ * GB

    in_copies = [
        pltpu.make_async_copy(src, dst, in_sems.at[i])
        for i, (src, dst) in enumerate([
            (x_hbm, x_ref), (wqkv_hbm, wqkv_ref), (wo_hbm, wo_ref),
            (w1_hbm, w1_ref), (b1_hbm, b1_ref), (w2_hbm, w2_ref)])
    ]
    for cp in in_copies:
        cp.start()

    def out_copy(t):
        rows = pl.ds(pl.multiple_of(t * TT, TT), TT)
        return pltpu.make_async_copy(x_ref.at[rows, :], out_hbm.at[rows, :], out_sems.at[t])

    def qkv_tile(t, carry):
        cols = pl.ds(pl.multiple_of(t * TT, TT), TT)
        xn = _ln_t(xt_ref[:, cols]).astype(bf16)
        qkv = jnp.dot(wqkvt_ref[...], xn, preferred_element_type=f32)
        qt_ref[:, cols] = (qkv[0:D] * (DH ** -0.5 * LOG2E)).astype(bf16)
        k_ref[cols, :] = qkv[D:2 * D].T.astype(bf16)
        vt_ref[:, cols] = qkv[2 * D:3 * D].astype(bf16)
        return carry

    def post_tile(t, layer):
        cols = pl.ds(pl.multiple_of(t * TT, TT), TT)
        x = xt_ref[:, cols] + jnp.dot(wot_ref[...], ot_ref[:, cols],
                                      preferred_element_type=f32)
        xn = _ln_t(x).astype(bf16)
        b = b1t_ref[...]
        h = jnp.dot(w1t_ref[...], xn, preferred_element_type=f32)
        h = h + jnp.concatenate([b] * (TT // 128), axis=1)
        act = _mish(h).astype(bf16)
        xt_ref[:, cols] = x + jnp.dot(w2t_ref[...], act, preferred_element_type=f32)

        @pl.when(layer == 1)
        def _():
            x_ref[cols, :] = xt_ref[:, cols].T.astype(bf16)
            out_copy(t).start()
        return layer

    def fused(ib, u, m_cur, s_buf, do1=True, do2=True):
        h = (ib % GB) * NB + u
        qt = ib // GB
        gn = (ib + 1) % GB
        hn = gn * NB + u
        qtn = (ib + 1) // GB
        if do1:
            qm = qt_ref[pl.ds(pl.multiple_of(hn * DH, DH), DH),
                        pl.ds(pl.multiple_of(qtn * TQ, TQ), TQ)]
        m = jnp.full((1, TQ), -jnp.inf, f32)
        o = jnp.zeros((DH, TQ), f32)
        l = jnp.zeros((1, TQ), f32)
        for c in range(NC):
            keys = pl.ds(c * KC, KC)
            if do2:
                pf = jnp.exp2(s_buf[keys, :] - m_cur)
                l = l + jnp.sum(pf, axis=0, keepdims=True)
                pb = pf.astype(bf16)
            if do1:
                kg = k_ref[keys, pl.ds(pl.multiple_of(gn * 128, 128), 128)]
                s = jnp.dot(kg[:, u * DH:(u + 1) * DH], qm, preferred_element_type=f32)
                s_buf[keys, :] = s
                m = jnp.maximum(m, jnp.max(s, axis=0, keepdims=True))
            if do2:
                o = o + jnp.dot(vt_ref[pl.ds(pl.multiple_of(h * DH, DH), DH), keys],
                                pb, preferred_element_type=f32)
        if do2:
            ot_ref[pl.ds(pl.multiple_of(h * DH, DH), DH),
                   pl.ds(pl.multiple_of(qt * TQ, TQ), TQ)] = (o / l).astype(bf16)
        return m

    def attention():
        ms = tuple(fused(-1, u, None, s_refs[u], do2=False) for u in range(NB))
        wot_ref[...] = wo_ref[...].astype(f32).T.astype(bf16)
        w1t_ref[...] = w1_ref[...].astype(f32).T.astype(bf16)
        w2t_ref[...] = w2_ref[...].astype(f32).T.astype(bf16)
        b1t_ref[...] = jnp.broadcast_to(b1_ref[...].astype(f32), (128, F)).T

        def body(ib, ms):
            return tuple(fused(ib, u, ms[u], s_refs[u]) for u in range(NB))

        ms = jax.lax.fori_loop(0, NBODY - 1, body, ms)
        for u in range(NB):
            fused(NBODY - 1, u, ms[u], s_refs[u], do1=False)

    in_copies[0].wait()
    for t in range(NT):
        xt_ref[:, t * TT:(t + 1) * TT] = x_ref[t * TT:(t + 1) * TT, :].astype(f32).T
    in_copies[1].wait()
    wqkvt_ref[...] = wqkv_ref[...].astype(f32).T.astype(bf16)

    def layer_fn(layer, carry):
        jax.lax.fori_loop(0, NT, qkv_tile, 0)

        @pl.when(layer == 0)
        def _():
            in_copies[2].wait()
            in_copies[3].wait()
            in_copies[4].wait()
            in_copies[5].wait()

        attention()
        jax.lax.fori_loop(0, NT, post_tile, layer)
        return carry

    jax.lax.fori_loop(0, 2, layer_fn, 0)
    for t in range(NT):
        out_copy(t).wait()


@jax.jit
def pallas_interleave_layers__mha_block__dense_activation_mish__prompt_kernel(
    A_x: jax.Array,
    A_wqkv: jax.Array,
    A_wo: jax.Array,
    B_x: jax.Array,
    B_w1: jax.Array,
    B_b1: jax.Array,
    B_w2: jax.Array,
):
    x = A_x.reshape(S, D)
    b1 = B_b1.reshape(1, F)
    out = pl.pallas_call(
        _kernel,
        out_shape=jax.ShapeDtypeStruct((S, D), bf16),
        in_specs=[pl.BlockSpec(memory_space=pl.ANY)] * 6,
        out_specs=pl.BlockSpec(memory_space=pl.ANY),
        scratch_shapes=[
            pltpu.VMEM((S, D), bf16),
            pltpu.VMEM((D, 3 * D), bf16),
            pltpu.VMEM((D, D), bf16),
            pltpu.VMEM((D, F), bf16),
            pltpu.VMEM((1, F), bf16),
            pltpu.VMEM((F, D), bf16),
            pltpu.SemaphoreType.DMA((6,)),
            pltpu.SemaphoreType.DMA((S // TT,)),
            pltpu.VMEM((D, S), f32),
            pltpu.VMEM((3 * D, D), bf16),
            pltpu.VMEM((D, D), bf16),
            pltpu.VMEM((F, D), bf16),
            pltpu.VMEM((D, F), bf16),
            pltpu.VMEM((F, 128), f32),
            pltpu.VMEM((D, S), bf16),
            pltpu.VMEM((S, D), bf16),
            pltpu.VMEM((D, S), bf16),
            pltpu.VMEM((D, S), bf16),
        ] + [pltpu.VMEM((S, TQ), f32) for _ in range(NB)],
        compiler_params=pltpu.CompilerParams(vmem_limit_bytes=100 * 1024 * 1024),
    )(x, A_wqkv, A_wo, B_w1, b1, B_w2)
    return out.reshape(1, S, D)
```

```python
import jax
import jax.numpy as jnp
import jax.experimental.pallas as pl
import jax.experimental.pallas.tpu as pltpu

S = 2048
D = 512
H = 32
DH = 16
F = 1792
EPS = 1e-5
LOG2E = 1.4426950408889634

TT = 1024
TQ = 256
KC = 256
NB = 8

f32 = jnp.float32
bf16 = jnp.bfloat16


def _ln_t(x):
    m = jnp.mean(x, axis=0, keepdims=True)
    xc = x - m
    v = jnp.mean(xc * xc, axis=0, keepdims=True)
    return xc * jax.lax.rsqrt(v + EPS)


def _mish(h):
    sp = jnp.log1p(jnp.exp(-jnp.abs(h))) + jnp.maximum(h, 0.0)
    return h * jnp.tanh(sp)


def _kernel(x_hbm, wqkv_hbm, wo_hbm, w1_hbm, b1_hbm, w2_hbm, out_hbm,
            x_ref, wqkv_ref, wo_ref, w1_ref, b1_ref, w2_ref, in_sems, out_sems,
            xt_ref, wqkvt_ref, wot_ref, w1t_ref, w2t_ref, b1t_ref,
            qt_ref, k_ref, vt_ref, ot_ref, *s_refs):
    NQ = S // TQ
    NC = S // KC
    NT = S // TT
    GB = H // NB
    NBODY = NQ * GB

    in_copies = [
        pltpu.make_async_copy(src, dst, in_sems.at[i])
        for i, (src, dst) in enumerate([
            (x_hbm, x_ref), (wqkv_hbm, wqkv_ref), (wo_hbm, wo_ref),
            (w1_hbm, w1_ref), (b1_hbm, b1_ref), (w2_hbm, w2_ref)])
    ]
    for cp in in_copies:
        cp.start()

    def out_copy(t):
        rows = pl.ds(pl.multiple_of(t * TT, TT), TT)
        return pltpu.make_async_copy(x_ref.at[rows, :], out_hbm.at[rows, :], out_sems.at[t])

    def qkv_tile(t, carry):
        cols = pl.ds(pl.multiple_of(t * TT, TT), TT)
        xn = _ln_t(xt_ref[:, cols]).astype(bf16)
        qkv = jnp.dot(wqkvt_ref[...], xn, preferred_element_type=f32)
        qt_ref[:, cols] = (qkv[0:D] * (DH ** -0.5 * LOG2E)).astype(bf16)
        k_ref[cols, :] = qkv[D:2 * D].T.astype(bf16)
        vt_ref[:, cols] = qkv[2 * D:3 * D].astype(bf16)
        return carry

    def post_tile(t, layer):
        cols = pl.ds(pl.multiple_of(t * TT, TT), TT)
        x = xt_ref[:, cols] + jnp.dot(wot_ref[...], ot_ref[:, cols],
                                      preferred_element_type=f32)
        xn = _ln_t(x).astype(bf16)
        b = b1t_ref[...]
        h = jnp.dot(w1t_ref[...], xn, preferred_element_type=f32)
        h = h + jnp.concatenate([b] * (TT // 128), axis=1)
        act = _mish(h).astype(bf16)
        xt_ref[:, cols] = x + jnp.dot(w2t_ref[...], act, preferred_element_type=f32)

        @pl.when(layer == 1)
        def _():
            x_ref[cols, :] = xt_ref[:, cols].T.astype(bf16)
            out_copy(t).start()
        return layer

    def fused(ib, u, m_cur, s_buf, do1=True, do2=True):
        h = (ib % GB) * NB + u
        qt = ib // GB
        gn = (ib + 1) % GB
        hn = gn * NB + u
        qtn = (ib + 1) // GB
        if do1:
            qm = qt_ref[pl.ds(pl.multiple_of(hn * DH, DH), DH),
                        pl.ds(pl.multiple_of(qtn * TQ, TQ), TQ)]
        m = jnp.full((8, TQ), -jnp.inf, f32)
        o = jnp.zeros((DH, TQ), f32)
        l = jnp.zeros((8, TQ), f32)
        for c in range(NC):
            keys = pl.ds(c * KC, KC)
            if do2:
                pf = jnp.exp2(s_buf[keys, :] - m_cur)
                l = l + jnp.sum(pf.reshape(KC // 8, 8, TQ), axis=0)
                pb = pf.astype(bf16)
            if do1:
                kg = k_ref[keys, pl.ds(pl.multiple_of(gn * 128, 128), 128)]
                s = jnp.dot(kg[:, u * DH:(u + 1) * DH], qm, preferred_element_type=f32)
                s_buf[keys, :] = s
                m = jnp.maximum(m, jnp.max(s.reshape(KC // 8, 8, TQ), axis=0))
            if do2:
                o = o + jnp.dot(vt_ref[pl.ds(pl.multiple_of(h * DH, DH), DH), keys],
                                pb, preferred_element_type=f32)
        if do2:
            ot_ref[pl.ds(pl.multiple_of(h * DH, DH), DH),
                   pl.ds(pl.multiple_of(qt * TQ, TQ), TQ)] = (o / jnp.sum(l, axis=0, keepdims=True)).astype(bf16)
        return jnp.max(m, axis=0, keepdims=True)

    def attention():
        ms = tuple(fused(-1, u, None, s_refs[u], do2=False) for u in range(NB))
        wot_ref[...] = wo_ref[...].astype(f32).T.astype(bf16)
        w1t_ref[...] = w1_ref[...].astype(f32).T.astype(bf16)
        w2t_ref[...] = w2_ref[...].astype(f32).T.astype(bf16)
        b1t_ref[...] = jnp.broadcast_to(b1_ref[...].astype(f32).reshape(1, F), (128, F)).T

        def body(ib, ms):
            return tuple(fused(ib, u, ms[u], s_refs[u]) for u in range(NB))

        ms = jax.lax.fori_loop(0, NBODY - 1, body, ms)
        for u in range(NB):
            fused(NBODY - 1, u, ms[u], s_refs[u], do1=False)

    in_copies[0].wait()
    for t in range(NT):
        xt_ref[:, t * TT:(t + 1) * TT] = x_ref[t * TT:(t + 1) * TT, :].astype(f32).T
    in_copies[1].wait()
    wqkvt_ref[...] = wqkv_ref[...].astype(f32).T.astype(bf16)

    def layer_fn(layer, carry):
        jax.lax.fori_loop(0, NT, qkv_tile, 0)

        @pl.when(layer == 0)
        def _():
            in_copies[2].wait()
            in_copies[3].wait()
            in_copies[4].wait()
            in_copies[5].wait()

        attention()
        jax.lax.fori_loop(0, NT, post_tile, layer)
        return carry

    jax.lax.fori_loop(0, 2, layer_fn, 0)
    for t in range(NT):
        out_copy(t).wait()


@jax.jit
def pallas_interleave_layers__mha_block__dense_activation_mish__prompt_kernel(
    A_x: jax.Array,
    A_wqkv: jax.Array,
    A_wo: jax.Array,
    B_x: jax.Array,
    B_w1: jax.Array,
    B_b1: jax.Array,
    B_w2: jax.Array,
):
    x = A_x.reshape(S, D)
    b1 = B_b1
    out = pl.pallas_call(
        _kernel,
        out_shape=jax.ShapeDtypeStruct((S, D), bf16),
        in_specs=[pl.BlockSpec(memory_space=pl.ANY)] * 6,
        out_specs=pl.BlockSpec(memory_space=pl.ANY),
        scratch_shapes=[
            pltpu.VMEM((S, D), bf16),
            pltpu.VMEM((D, 3 * D), bf16),
            pltpu.VMEM((D, D), bf16),
            pltpu.VMEM((D, F), bf16),
            pltpu.VMEM((F,), bf16),
            pltpu.VMEM((F, D), bf16),
            pltpu.SemaphoreType.DMA((6,)),
            pltpu.SemaphoreType.DMA((S // TT,)),
            pltpu.VMEM((D, S), f32),
            pltpu.VMEM((3 * D, D), bf16),
            pltpu.VMEM((D, D), bf16),
            pltpu.VMEM((F, D), bf16),
            pltpu.VMEM((D, F), bf16),
            pltpu.VMEM((F, 128), f32),
            pltpu.VMEM((D, S), bf16),
            pltpu.VMEM((S, D), bf16),
            pltpu.VMEM((D, S), bf16),
            pltpu.VMEM((D, S), bf16),
        ] + [pltpu.VMEM((S, TQ), f32) for _ in range(NB)],
        compiler_params=pltpu.CompilerParams(vmem_limit_bytes=100 * 1024 * 1024),
    )(x, A_wqkv, A_wo, B_w1, b1, B_w2)
    return out.reshape(1, S, D)
```
